```python
import jax
import jax.numpy as jnp

def _softmax(x, axis=-1):
    return jax.nn.softmax(x, axis=axis)
def _gelu(x):
    return jax.nn.gelu(x, approximate=True)
def _silu(x):
    return jax.nn.silu(x)
def _sigmoid(x):
    return jax.nn.sigmoid(x)
def _layernorm(x, axis=-1, eps=1e-5):
    m = jnp.mean(x, axis=axis, keepdims=True)
    v = jnp.var(x, axis=axis, keepdims=True)
    return (x - m) / jnp.sqrt(v + eps)
def _scatter_add(tgt, idx, src, axis=0):
    return tgt.at[idx].add(src)
def _segment_sum(src, seg, n):
    return jax.ops.segment_sum(src, seg, n)
class _Rng:
    def __init__(self, key):
        self._k = key
    def _next(self):
        self._k, sub = jax.random.split(self._k)
        return sub
    def normal(self, shape):
        return jax.random.normal(self._next(), shape, dtype=jnp.bfloat16)
    def randint(self, lo, hi, shape):
        return jax.random.randint(self._next(), shape, lo, hi, dtype=jnp.int32)
    def uniform(self, shape, lo=0.0, hi=1.0):
        return jax.random.uniform(self._next(), shape, jnp.bfloat16, lo, hi)
    def permutation(self, n):
        return jax.random.permutation(self._next(), n)


kernel_name = 'recurrent_scan__sliding_block_cached__glu_gated_swiglu__decode'

def setup_inputs():
    _rng = _Rng(jax.random.key(int.from_bytes(__import__("os").urandom(4), "little")))
    _w = (lambda a: (lambda t: t.astype(jnp.bfloat16) if jnp.issubdtype(t.dtype, jnp.floating) else t)(jnp.asarray(a)))
    def _A_setup():
        B, Sq, D = 1, 1, 640
        Hq, Hkv, Sk, Dh = 32, 32, 32768, 192
        assert Hq % Hkv == 0, (Hq, Hkv)
        return {
            "x": _w((lambda *s: _rng.normal(s) * 0.05)(B, Sq, D)),
            "k_cache": _w((lambda *s: _rng.normal(s) * 0.05)(B, Hkv, Sk, Dh)),
            "v_cache": _w((lambda *s: _rng.normal(s) * 0.05)(B, Hkv, Sk, Dh)),
            "wq": _w((lambda *s: _rng.normal(s) * 0.05)(D, Hq * Dh) * (D ** -0.5)),
            "wo": _w((lambda *s: _rng.normal(s) * 0.05)(Hq * Dh, D) * ((Hq * Dh) ** -0.5)),
        }
    _A_in = _A_setup()

    def _B_setup():
        B, S, D, F = 1, 1, 640, 1536
        return {
            "x": _w((lambda *s: _rng.normal(s) * 0.05)(B, S, D)),
            "w1": _w((lambda *s: _rng.normal(s) * 0.05)(D, F) * (2.0 / D) ** 0.5),
            "w3": _w((lambda *s: _rng.normal(s) * 0.05)(D, F) * (2.0 / D) ** 0.5),
            "w2": _w((lambda *s: _rng.normal(s) * 0.05)(F, D) * (2.0 / F) ** 0.5),
        }
    _B_in = _B_setup()

    return {
        "A_x": _A_in["x"],
        "A_k_cache": _A_in["k_cache"],
        "A_v_cache": _A_in["v_cache"],
        "A_wq": _A_in["wq"],
        "A_wo": _A_in["wo"],
        "B_x": _B_in["x"],
        "B_w1": _B_in["w1"],
        "B_w3": _B_in["w3"],
        "B_w2": _B_in["w2"],
    }

def reference(A_x, A_k_cache, A_v_cache, A_wq, A_wo, B_x, B_w1, B_w3, B_w2):
    def _A_ref(x, k_cache, v_cache, wq, wo):
        B, Sq, D = x.shape
        Hq, Dh = 32, 192
        Hkv, Sk = k_cache.shape[1], k_cache.shape[2]
        W = min(4096, max(256, Sk // 4))
        rep = Hq // Hkv
        q = (lambda x, *d: x.transpose(*d))((x @ wq).reshape(B, Sq, Hq, Dh), 0, 2, 1, 3)
        k = jnp.repeat(k_cache[:, :, Sk - W:, :], rep, axis=1)
        v = jnp.repeat(v_cache[:, :, Sk - W:, :], rep, axis=1)
        scores = jnp.einsum("bhqd,bhkd->bhqk", q, k) * (Dh ** -0.5)
        p = _softmax(scores, axis=-1)
        o = jnp.einsum("bhqk,bhkd->bhqd", p, v)
        return (lambda x, *d: x.transpose(*d))(o, 0, 2, 1, 3).reshape(B, Sq, Hq * Dh) @ wo

    def _B_ref(x, w1, w3, w2):
        gate = jnp.einsum("bsd,df->bsf", x, w1)
        up = jnp.einsum("bsd,df->bsf", x, w3)
        h = _silu(gate) * up
        out = jnp.einsum("bsf,fd->bsd", h, w2)
        return out

    x = A_x
    xn = _layernorm(x, axis=-1)
    s = _A_ref(xn, A_k_cache, A_v_cache, A_wq, A_wo)
    g = _silu(_B_ref(xn, B_w1, B_w3, B_w2))
    return x + s * g
```

```python
import functools

import jax
import jax.numpy as jnp
import jax.experimental.pallas as pl
import jax.experimental.pallas.tpu as pltpu

BF16 = jnp.bfloat16
F32 = jnp.float32

LANE = 128
ROWS = 8
EPS = 1e-5
NSLOT = 3
NW2 = 4
EARLY = (5, 5, 5)


def _silu(v):
    return v * jax.nn.sigmoid(v)


def _kernel(x_hbm, k_hbm, v_hbm, wq_hbm, wo_hbm, w1_hbm, w3_hbm, w2_hbm,
            out_ref,
            x_v, kbuf, vbuf, wq_v, wo_v, w1_v, w3_v, w2_v, q_s, o_s,
            sem_x, sem_wq, sem_w13, sem_k, sem_v, sem_wo, sem_w2,
            *, dims):
    D, H, DH, SK, W, FF = dims
    scale = float(DH) ** -0.5
    HH = H // 2

    def wait_all(region, sem):
        pltpu.make_async_copy(region, region, sem).wait()

    def start_pair(src0, dst0, sem0, r0, src1, dst1, sem1, r1, nrows, rb, cb):
        ncols = src0.shape[1]

        def body(i, carry):
            ra = pl.multiple_of(r0 + i * rb, 8)
            rb_ = pl.multiple_of(r1 + i * rb, 8)
            for c in range(0, ncols, cb):
                pltpu.make_async_copy(src0.at[pl.ds(ra, rb), pl.ds(c, cb)],
                                      dst0.at[pl.ds(ra, rb), pl.ds(c, cb)], sem0).start(priority=0)
                pltpu.make_async_copy(src1.at[pl.ds(rb_, rb), pl.ds(c, cb)],
                                      dst1.at[pl.ds(rb_, rb), pl.ds(c, cb)], sem1).start(priority=1)
            return carry

        jax.lax.fori_loop(0, nrows // rb, body, 0)

    def start_kv(h, slot):
        def body(i, carry):
            c = pl.multiple_of(i * LANE, LANE)
            pltpu.make_async_copy(k_hbm.at[0, h, :, pl.ds(SK - W + c, LANE)],
                                  kbuf.at[slot, :, pl.ds(c, LANE)], sem_k.at[slot]).start(priority=0)
            pltpu.make_async_copy(v_hbm.at[0, h, :, pl.ds(SK - W + c, LANE)],
                                  vbuf.at[slot, :, pl.ds(c, LANE)], sem_v.at[slot]).start(priority=1)
            return carry

        jax.lax.fori_loop(0, W // LANE, body, 0)

    def start_wo(g):
        start_pair(wo_hbm, wo_v, sem_wo.at[0, g], g * DH, wo_hbm, wo_v, sem_wo.at[1, g], (g + HH) * DH,
                   DH, 32, D)

    def start_tail_item(i):
        if i < NW2:
            n = FF // 2 // NW2
            start_pair(w2_hbm, w2_v, sem_w2.at[0], i * n, w2_hbm, w2_v, sem_w2.at[1], FF // 2 + i * n,
                       n, 32, D)
        else:
            start_wo(i - NW2)

    x_copy = pltpu.make_async_copy(x_hbm, x_v, sem_x)
    x_copy.start()
    start_pair(wq_hbm, wq_v, sem_wq.at[0], 0, wq_hbm, wq_v, sem_wq.at[1], D // 2, D // 2, 8, H * DH // 2)
    start_pair(w1_hbm, w1_v, sem_w13.at[0], 0, w3_hbm, w3_v, sem_w13.at[1], 0, D, 16, FF)
    start_kv(0, 0)

    x_copy.wait()
    x = x_v[0].astype(F32)
    mean = jnp.mean(x, axis=-1, keepdims=True)
    xc = x - mean
    var = jnp.mean(xc * xc, axis=-1, keepdims=True)
    xn = xc / jnp.sqrt(var + EPS)
    xn8 = jnp.broadcast_to(xn, (ROWS, D)).astype(BF16)

    wait_all(wq_v.at[pl.ds(0, D // 2)], sem_wq.at[0])
    wait_all(wq_v.at[pl.ds(D // 2, D // 2)], sem_wq.at[1])
    for hp in range(HH):
        qq = jnp.dot(xn8, wq_v[:, hp * 2 * DH:(hp + 1) * 2 * DH], preferred_element_type=F32)
        q_s[2 * hp] = qq[:, :DH].astype(BF16)
        q_s[2 * hp + 1] = qq[:, DH:].astype(BF16)
    start_kv(1, 1)

    wait_all(w1_v, sem_w13.at[0])
    wait_all(w3_v, sem_w13.at[1])
    gate = jnp.dot(xn8, w1_v[...], preferred_element_type=F32)
    up = jnp.dot(xn8, w3_v[...], preferred_element_type=F32)
    hid = (_silu(gate) * up).astype(BF16)
    for h in range(2, NSLOT):
        start_kv(h, h)

    def head_body(h, carry):
        slot = h % NSLOT
        wait_all(kbuf.at[slot], sem_k.at[slot])
        s = jnp.dot(q_s[h], kbuf[slot], preferred_element_type=F32) * scale
        m = jnp.max(s, axis=-1, keepdims=True)
        p = jnp.exp(s - m)
        l = jnp.sum(p, axis=-1, keepdims=True)
        wait_all(vbuf.at[slot], sem_v.at[slot])
        o = jax.lax.dot_general(p.astype(BF16), vbuf[slot], (((1,), (1,)), ((), ())),
                                preferred_element_type=F32)
        o_s[h] = (o / l).astype(BF16)

        @pl.when(h + NSLOT < H)
        def _():
            start_kv(h + NSLOT, slot)

        first = 0
        for j, n in enumerate(EARLY):
            @pl.when(h == H - NSLOT + j)
            def _(first=first, n=n):
                for i in range(first, first + n):
                    start_tail_item(i)
            first += n
        return carry

    jax.lax.fori_loop(0, H, head_body, 0)

    wait_all(w2_v.at[pl.ds(0, FF // 2)], sem_w2.at[0])
    wait_all(w2_v.at[pl.ds(FF // 2, FF // 2)], sem_w2.at[1])
    gate_out = _silu(jnp.dot(hid, w2_v[...], preferred_element_type=F32))

    issued = sum(EARLY) - NW2

    def wo_body(g, acc):
        @pl.when(g + issued < HH)
        def _():
            start_wo(g + issued)

        for half in range(2):
            r0 = pl.multiple_of((half * HH + g) * DH, DH)
            wait_all(wo_v.at[pl.ds(r0, DH)], sem_wo.at[half, g])
        for half in range(2):
            h = half * HH + g
            r0 = pl.multiple_of(h * DH, DH)
            acc = acc + jnp.dot(o_s[h], wo_v[pl.ds(r0, DH), :], preferred_element_type=F32)
        return acc

    attn = jax.lax.fori_loop(0, HH, wo_body, jnp.zeros((ROWS, D), F32))

    out_ref[0] = (x + attn[0:1] * gate_out[0:1]).astype(out_ref.dtype)


@jax.jit
def pallas_recurrent_scan__sliding_block_cached__glu_gated_swiglu__decode_kernel(
    A_x: jax.Array,
    A_k_cache: jax.Array,
    A_v_cache: jax.Array,
    A_wq: jax.Array,
    A_wo: jax.Array,
    B_x: jax.Array,
    B_w1: jax.Array,
    B_w3: jax.Array,
    B_w2: jax.Array,
):
    del B_x
    B, SQ, D = A_x.shape
    _, H, SK, DH = A_k_cache.shape
    FF = B_w1.shape[1]
    assert B == 1 and SQ == 1
    W = min(4096, max(256, SK // 4))

    kt = jnp.swapaxes(A_k_cache, 2, 3)
    vt = jnp.swapaxes(A_v_cache, 2, 3)

    kernel = functools.partial(_kernel, dims=(D, H, DH, SK, W, FF))
    in_hbm = pl.BlockSpec(memory_space=pl.ANY)
    return pl.pallas_call(
        kernel,
        out_shape=jax.ShapeDtypeStruct((B, SQ, D), A_x.dtype),
        in_specs=[in_hbm] * 8,
        out_specs=pl.BlockSpec(memory_space=pltpu.VMEM),
        scratch_shapes=[
            pltpu.VMEM((B, SQ, D), BF16),
            pltpu.VMEM((NSLOT, DH, W), BF16),
            pltpu.VMEM((NSLOT, DH, W), BF16),
            pltpu.VMEM((D, H * DH), BF16),
            pltpu.VMEM((H * DH, D), BF16),
            pltpu.VMEM((D, FF), BF16),
            pltpu.VMEM((D, FF), BF16),
            pltpu.VMEM((FF, D), BF16),
            pltpu.VMEM((H, ROWS, DH), BF16),
            pltpu.VMEM((H, ROWS, DH), BF16),
            pltpu.SemaphoreType.DMA,
            pltpu.SemaphoreType.DMA((2,)),
            pltpu.SemaphoreType.DMA((2,)),
            pltpu.SemaphoreType.DMA((NSLOT,)),
            pltpu.SemaphoreType.DMA((NSLOT,)),
            pltpu.SemaphoreType.DMA((2, H // 2)),
            pltpu.SemaphoreType.DMA((2,)),
        ],
        compiler_params=pltpu.CompilerParams(
            vmem_limit_bytes=64 * 1024 * 1024,
            disable_bounds_checks=True,
            disable_semaphore_checks=True,
        ),
    )(A_x, kt, vt, A_wq, A_wo, B_w1, B_w3, B_w2)
```

```python
import functools

import jax
import jax.numpy as jnp
import jax.experimental.pallas as pl
import jax.experimental.pallas.tpu as pltpu

BF16 = jnp.bfloat16
F32 = jnp.float32

LANE = 128
ROWS = 8
EPS = 1e-5
NSLOT = 3
NW2 = 4
EARLY = (5, 5, 5)
WQ_FIRST = 24


def _silu(v):
    return v * jax.nn.sigmoid(v)


def _kernel(x_hbm, k_hbm, v_hbm, wq_hbm, wo_hbm, w1_hbm, w3_hbm, w2_hbm,
            out_ref,
            x_v, kbuf, vbuf, wq_v, wo_v, w1_v, w3_v, w2_v, q_s, o_s,
            sem_x, sem_wq, sem_w13, sem_k, sem_v, sem_wo, sem_w2,
            *, dims):
    D, H, DH, SK, W, FF = dims
    scale = float(DH) ** -0.5
    HH = H // 2

    def wait_all(region, sem):
        pltpu.make_async_copy(region, region, sem).wait()

    def start_pair(src0, dst0, sem0, r0, src1, dst1, sem1, r1, nrows, rb, cb):
        ncols = src0.shape[1]

        def body(i, carry):
            ra = pl.multiple_of(r0 + i * rb, 8)
            rb_ = pl.multiple_of(r1 + i * rb, 8)
            for c in range(0, ncols, cb):
                pltpu.make_async_copy(src0.at[pl.ds(ra, rb), pl.ds(c, cb)],
                                      dst0.at[pl.ds(ra, rb), pl.ds(c, cb)], sem0).start(priority=0)
                pltpu.make_async_copy(src1.at[pl.ds(rb_, rb), pl.ds(c, cb)],
                                      dst1.at[pl.ds(rb_, rb), pl.ds(c, cb)], sem1).start(priority=1)
            return carry

        jax.lax.fori_loop(0, nrows // rb, body, 0)

    def start_kv(h, slot):
        def body(i, carry):
            c = pl.multiple_of(i * LANE, LANE)
            pltpu.make_async_copy(k_hbm.at[0, h, :, pl.ds(SK - W + c, LANE)],
                                  kbuf.at[slot, :, pl.ds(c, LANE)], sem_k.at[slot]).start(priority=0)
            pltpu.make_async_copy(v_hbm.at[0, h, :, pl.ds(SK - W + c, LANE)],
                                  vbuf.at[slot, :, pl.ds(c, LANE)], sem_v.at[slot]).start(priority=1)
            return carry

        jax.lax.fori_loop(0, W // LANE, body, 0)

    def start_wo(g):
        start_pair(wo_hbm, wo_v, sem_wo.at[0, g], g * DH, wo_hbm, wo_v, sem_wo.at[1, g], (g + HH) * DH,
                   DH, 32, D)

    def start_tail_item(i):
        if i < NW2:
            n = FF // 2 // NW2
            start_pair(w2_hbm, w2_v, sem_w2.at[0], i * n, w2_hbm, w2_v, sem_w2.at[1], FF // 2 + i * n,
                       n, 32, D)
        else:
            start_wo(i - NW2)

    x_copy = pltpu.make_async_copy(x_hbm, x_v, sem_x)
    x_copy.start()
    start_pair(wq_hbm, wq_v, sem_wq.at[0], 0, wq_hbm, wq_v, sem_wq.at[1], D // 2, WQ_FIRST, 8, 512)
    start_pair(wq_hbm, wq_v, sem_wq.at[0], WQ_FIRST, wq_hbm, wq_v, sem_wq.at[1], D // 2 + WQ_FIRST,
               D // 2 - WQ_FIRST, 8, H * DH // 2)
    start_pair(w1_hbm, w1_v, sem_w13.at[0], 0, w3_hbm, w3_v, sem_w13.at[1], 0, D, 16, FF)
    start_kv(0, 0)

    x_copy.wait()
    x = x_v[0].astype(F32)
    mean = jnp.mean(x, axis=-1, keepdims=True)
    xc = x - mean
    var = jnp.mean(xc * xc, axis=-1, keepdims=True)
    xn = xc / jnp.sqrt(var + EPS)
    xn8 = jnp.broadcast_to(xn, (ROWS, D)).astype(BF16)

    wait_all(wq_v.at[pl.ds(0, D // 2)], sem_wq.at[0])
    wait_all(wq_v.at[pl.ds(D // 2, D // 2)], sem_wq.at[1])
    for hp in range(HH):
        qq = jnp.dot(xn8, wq_v[:, hp * 2 * DH:(hp + 1) * 2 * DH], preferred_element_type=F32)
        q_s[2 * hp] = qq[:, :DH].astype(BF16)
        q_s[2 * hp + 1] = qq[:, DH:].astype(BF16)
    start_kv(1, 1)

    wait_all(w1_v, sem_w13.at[0])
    wait_all(w3_v, sem_w13.at[1])
    gate = jnp.dot(xn8, w1_v[...], preferred_element_type=F32)
    up = jnp.dot(xn8, w3_v[...], preferred_element_type=F32)
    hid = (_silu(gate) * up).astype(BF16)
    for h in range(2, NSLOT):
        start_kv(h, h)

    def head_body(h, carry):
        slot = h % NSLOT
        wait_all(kbuf.at[slot], sem_k.at[slot])
        s = jnp.dot(q_s[h], kbuf[slot], preferred_element_type=F32) * scale
        m = jnp.max(s, axis=-1, keepdims=True)
        p = jnp.exp(s - m)
        l = jnp.sum(p, axis=-1, keepdims=True)
        wait_all(vbuf.at[slot], sem_v.at[slot])
        o = jax.lax.dot_general(p.astype(BF16), vbuf[slot], (((1,), (1,)), ((), ())),
                                preferred_element_type=F32)
        o_s[h] = (o / l).astype(BF16)

        @pl.when(h + NSLOT < H)
        def _():
            start_kv(h + NSLOT, slot)

        first = 0
        for j, n in enumerate(EARLY):
            @pl.when(h == H - NSLOT + j)
            def _(first=first, n=n):
                for i in range(first, first + n):
                    start_tail_item(i)
            first += n
        return carry

    jax.lax.fori_loop(0, H, head_body, 0)

    wait_all(w2_v.at[pl.ds(0, FF // 2)], sem_w2.at[0])
    wait_all(w2_v.at[pl.ds(FF // 2, FF // 2)], sem_w2.at[1])
    gate_out = _silu(jnp.dot(hid, w2_v[...], preferred_element_type=F32))

    issued = sum(EARLY) - NW2

    def wo_body(g, acc):
        @pl.when(g + issued < HH)
        def _():
            start_wo(g + issued)

        for half in range(2):
            r0 = pl.multiple_of((half * HH + g) * DH, DH)
            wait_all(wo_v.at[pl.ds(r0, DH)], sem_wo.at[half, g])
        for half in range(2):
            h = half * HH + g
            r0 = pl.multiple_of(h * DH, DH)
            acc = acc + jnp.dot(o_s[h], wo_v[pl.ds(r0, DH), :], preferred_element_type=F32)
        return acc

    attn = jax.lax.fori_loop(0, HH, wo_body, jnp.zeros((ROWS, D), F32))

    out_ref[0] = (x + attn[0:1] * gate_out[0:1]).astype(out_ref.dtype)


@jax.jit
def pallas_recurrent_scan__sliding_block_cached__glu_gated_swiglu__decode_kernel(
    A_x: jax.Array,
    A_k_cache: jax.Array,
    A_v_cache: jax.Array,
    A_wq: jax.Array,
    A_wo: jax.Array,
    B_x: jax.Array,
    B_w1: jax.Array,
    B_w3: jax.Array,
    B_w2: jax.Array,
):
    del B_x
    B, SQ, D = A_x.shape
    _, H, SK, DH = A_k_cache.shape
    FF = B_w1.shape[1]
    assert B == 1 and SQ == 1
    W = min(4096, max(256, SK // 4))

    kt = jnp.swapaxes(A_k_cache, 2, 3)
    vt = jnp.swapaxes(A_v_cache, 2, 3)

    kernel = functools.partial(_kernel, dims=(D, H, DH, SK, W, FF))
    in_hbm = pl.BlockSpec(memory_space=pl.ANY)
    return pl.pallas_call(
        kernel,
        out_shape=jax.ShapeDtypeStruct((B, SQ, D), A_x.dtype),
        in_specs=[in_hbm] * 8,
        out_specs=pl.BlockSpec(memory_space=pltpu.VMEM),
        scratch_shapes=[
            pltpu.VMEM((B, SQ, D), BF16),
            pltpu.VMEM((NSLOT, DH, W), BF16),
            pltpu.VMEM((NSLOT, DH, W), BF16),
            pltpu.VMEM((D, H * DH), BF16),
            pltpu.VMEM((H * DH, D), BF16),
            pltpu.VMEM((D, FF), BF16),
            pltpu.VMEM((D, FF), BF16),
            pltpu.VMEM((FF, D), BF16),
            pltpu.VMEM((H, ROWS, DH), BF16),
            pltpu.VMEM((H, ROWS, DH), BF16),
            pltpu.SemaphoreType.DMA,
            pltpu.SemaphoreType.DMA((2,)),
            pltpu.SemaphoreType.DMA((2,)),
            pltpu.SemaphoreType.DMA((NSLOT,)),
            pltpu.SemaphoreType.DMA((NSLOT,)),
            pltpu.SemaphoreType.DMA((2, H // 2)),
            pltpu.SemaphoreType.DMA((2,)),
        ],
        compiler_params=pltpu.CompilerParams(
            vmem_limit_bytes=64 * 1024 * 1024,
            disable_bounds_checks=True,
            disable_semaphore_checks=True,
        ),
    )(A_x, kt, vt, A_wq, A_wo, B_w1, B_w3, B_w2)
```
